```python
import os as _os
_os.environ.setdefault("JAX_PLATFORMS", "cpu")
import jax
import jax.numpy as jnp

def _softmax(x, axis=-1):
    return jax.nn.softmax(x, axis=axis)
def _gelu(x):
    return jax.nn.gelu(x, approximate=True)
def _silu(x):
    return jax.nn.silu(x)
def _sigmoid(x):
    return jax.nn.sigmoid(x)
def _layernorm(x, axis=-1, eps=1e-5):
    m = jnp.mean(x, axis=axis, keepdims=True)
    v = jnp.var(x, axis=axis, keepdims=True)
    return (x - m) / jnp.sqrt(v + eps)
def _scatter_add(tgt, idx, src, axis=0):
    return tgt.at[idx].add(src)
def _segment_sum(src, seg, n):
    return jax.ops.segment_sum(src, seg, n)
class _Rng:
    def __init__(self, key):
        self._k = key
    def _next(self):
        self._k, sub = jax.random.split(self._k)
        return sub
    def normal(self, shape):
        return jax.random.normal(self._next(), shape, dtype=jnp.bfloat16)
    def randint(self, lo, hi, shape):
        return jax.random.randint(self._next(), shape, lo, hi, dtype=jnp.int32)
    def uniform(self, shape, lo=0.0, hi=1.0):
        return jax.random.uniform(self._next(), shape, jnp.bfloat16, lo, hi)
    def permutation(self, n):
        return jax.random.permutation(self._next(), n)


kernel_name = 'concat_heads__mha_block_cached__mha_block_cached__near_ridge'

def setup_inputs():
    _rng = _Rng(jax.random.key(int.from_bytes(__import__("os").urandom(4), "little")))
    _w = (lambda a: (lambda t: t.astype(jnp.bfloat16) if jnp.issubdtype(t.dtype, jnp.floating) else t)(jnp.asarray(a)))
    def _A_setup():
        B, Sq, D = 8, 160, 512
        H, Sk, Dh = 32, 512, 128
        return {
            "x": _w((lambda *s: _rng.normal(s) * 0.8)(B, Sq, D)),
            "k_cache": _w((lambda *s: _rng.normal(s) * 0.8)(B, H, Sk, Dh)),
            "v_cache": _w((lambda *s: _rng.normal(s) * 0.05)(B, H, Sk, Dh)),
            "wq": _w((lambda *s: _rng.normal(s) * 0.8)(D, H * Dh) * (D ** -0.5)),
            "wo": _w((lambda *s: _rng.normal(s) * 0.05)(H * Dh, D) * ((H * Dh) ** -0.5)),
        }
    _A_in = _A_setup()

    def _B_setup():
        B, Sq, D = 8, 160, 512
        H, Sk, Dh = 32, 512, 128
        return {
            "x": _w((lambda *s: _rng.normal(s) * 0.8)(B, Sq, D)),
            "k_cache": _w((lambda *s: _rng.normal(s) * 0.8)(B, H, Sk, Dh)),
            "v_cache": _w((lambda *s: _rng.normal(s) * 0.05)(B, H, Sk, Dh)),
            "wq": _w((lambda *s: _rng.normal(s) * 0.8)(D, H * Dh) * (D ** -0.5)),
            "wo": _w((lambda *s: _rng.normal(s) * 0.05)(H * Dh, D) * ((H * Dh) ** -0.5)),
        }
    _B_in = _B_setup()

    return {
        "A_x": _A_in["x"],
        "A_k_cache": _A_in["k_cache"],
        "A_v_cache": _A_in["v_cache"],
        "A_wq": _A_in["wq"],
        "A_wo": _A_in["wo"],
        "B_x": _B_in["x"],
        "B_k_cache": _B_in["k_cache"],
        "B_v_cache": _B_in["v_cache"],
        "B_wq": _B_in["wq"],
        "B_wo": _B_in["wo"],
    }

def reference(A_x, A_k_cache, A_v_cache, A_wq, A_wo, B_x, B_k_cache, B_v_cache, B_wq, B_wo):
    def _A_ref(x, k_cache, v_cache, wq, wo):
        B, Sq, D = x.shape
        H, Dh = 32, 128
        q = (lambda x, *d: x.transpose(*d))((x @ wq).reshape(B, Sq, H, Dh), 0, 2, 1, 3)
        scores = jnp.einsum("bhqd,bhkd->bhqk", q, k_cache) * (Dh ** -0.5)
        p = _softmax(scores, axis=-1)
        o = jnp.einsum("bhqk,bhkd->bhqd", p, v_cache)
        return (lambda x, *d: x.transpose(*d))(o, 0, 2, 1, 3).reshape(B, Sq, H * Dh) @ wo

    def _B_ref(x, k_cache, v_cache, wq, wo):
        B, Sq, D = x.shape
        H, Dh = 32, 128
        q = (lambda x, *d: x.transpose(*d))((x @ wq).reshape(B, Sq, H, Dh), 0, 2, 1, 3)
        scores = jnp.einsum("bhqd,bhkd->bhqk", q, k_cache) * (Dh ** -0.5)
        p = _softmax(scores, axis=-1)
        o = jnp.einsum("bhqk,bhkd->bhqd", p, v_cache)
        return (lambda x, *d: x.transpose(*d))(o, 0, 2, 1, 3).reshape(B, Sq, H * Dh) @ wo

    a = _A_ref(A_x, A_k_cache, A_v_cache, A_wq, A_wo)
    b = _B_ref(B_x, B_k_cache, B_v_cache, B_wq, B_wo)
    return jnp.concatenate([a, b], axis=-1)
```

```python
import jax
import jax.numpy as jnp
from jax import lax
import jax.experimental.pallas as pl
import jax.experimental.pallas.tpu as pltpu

B, SQ, D, H, SK, DH = 8, 160, 512, 32, 512, 128
M = B * SQ
NSTEP = 2 * H
LOG2E = 1.4426950408889634
QSCALE = (DH ** -0.5) * LOG2E

U = 5
NBUF = 5
LA = 3
A = 4
T = 4
XCH = 4
NMAIN = NSTEP - T
XR = M // XCH
assert U % NBUF == 0 and NMAIN % U == 0 and A <= T and A < U and LA < NBUF

f32 = jnp.float32
bf16 = jnp.bfloat16


def _kernel(ax, ak, av, awq, awo, bx, bk, bv, bwq, bwo, out_ref, *scratch):
    scratch = list(scratch)
    take = lambda n: [scratch.pop(0) for _ in range(n)]
    x_buf, acc, ostage, wq0_buf, q_scr = take(5)
    k_buf, v_buf, wq_buf, wo_buf = take(NBUF), take(NBUF), take(NBUF), take(NBUF)
    o_scr = take(2)
    x_sem, k_sem, v_sem, wq_sem, wo_sem, wq0_sem, o_sem = take(7)
    srcs = ((ak, av, awq, awo), (bk, bv, bwq, bwo))

    def kvo_copies(br, h, slot):
        k, v, _, wo = srcs[br]
        rows = pl.ds(pl.multiple_of(h * DH, DH), DH)
        return (
            pltpu.make_async_copy(k.at[:, h], k_buf[slot], k_sem.at[slot]),
            pltpu.make_async_copy(v.at[:, h], v_buf[slot], v_sem.at[slot]),
            pltpu.make_async_copy(wo.at[rows, :], wo_buf[slot], wo_sem.at[slot]),
        )

    def wq_copy(br, h, dst, sem):
        cols = pl.ds(pl.multiple_of(h * DH, DH), DH)
        return pltpu.make_async_copy(srcs[br][2].at[:, cols], dst, sem)

    def start_group(j, slot):
        jq = j + A
        if isinstance(j, int):
            if j < NSTEP:
                for c in kvo_copies(j // H, j % H, slot):
                    c.start()
            if jq < NSTEP:
                wq_copy(jq // H, jq % H, wq_buf[slot], wq_sem.at[slot]).start()
            return
        for br in range(2):
            @pl.when((j >> 5) == br)
            def _():
                for c in kvo_copies(br, j & (H - 1), slot):
                    c.start()
        for br in range(2):
            @pl.when((jq >> 5) == br)
            def _():
                wq_copy(br, jq & (H - 1), wq_buf[slot], wq_sem.at[slot]).start()

    def wait_group(j, slot):
        for c in kvo_copies(0, 0, slot):
            c.wait()
        if not isinstance(j, int) or j + A < NSTEP:
            wq_copy(0, 0, wq_buf[slot], wq_sem.at[slot]).wait()

    def out_copy(br, b):
        rows = pl.ds(b * SQ, SQ)
        return pltpu.make_async_copy(
            ostage.at[br, rows, :], out_ref.at[rows, pl.ds(br * D, D)], o_sem.at[br * B + b])

    xa_copies = [
        pltpu.make_async_copy(ax.at[pl.ds(c * XR, XR), :], x_buf.at[0, pl.ds(c * XR, XR), :],
                              x_sem.at[c])
        for c in range(XCH)
    ]
    xb_copy = pltpu.make_async_copy(bx, x_buf.at[1], x_sem.at[XCH])
    wq0_copy = lambda a: wq_copy(0, a, wq0_buf.at[a], wq0_sem.at[a])

    def issue(i, carry):
        @pl.when(i == 0)
        def _():
            wq0_copy(0).start()
            for c in xa_copies:
                c.start()
            for a in range(1, A):
                wq0_copy(a).start()
        for j in range(LA):
            @pl.when(i == j + 1)
            def _():
                start_group(j, j)
        return carry

    lax.fori_loop(0, LA + 1, issue, 0)

    def q_ahead(a, carry):
        wq0_copy(a).wait()
        for c in range(XCH):
            @pl.when(a == 0)
            def _():
                xa_copies[c].wait()
            q = jnp.dot(x_buf[0, c * XR:(c + 1) * XR, :], wq0_buf[a], preferred_element_type=f32)
            q_scr[a, c * XR:(c + 1) * XR, :] = (q * QSCALE).astype(bf16)
        return carry

    lax.fori_loop(0, A, q_ahead, 0)

    def step(j, u, last=False):
        slot = u % NBUF
        par = u % 2
        static = isinstance(j, int)
        wait_group(j, slot)
        start_group(j + LA, (u + LA) % NBUF)
        br = j // H if static else j >> 5

        def qproj():
            nbr = (j + A) // H if static else (j + A) >> 5
            q = jnp.dot(x_buf[nbr], wq_buf[slot][...], preferred_element_type=f32)
            q_scr[(u + A) % U] = (q * QSCALE).astype(bf16)

        def scores(b):
            return lax.dot_general(q_scr[u, b * SQ:(b + 1) * SQ, :], k_buf[slot][b],
                                   (((1,), (1,)), ((), ())), preferred_element_type=f32)

        def pv(b, s):
            m = jnp.max(s, axis=-1, keepdims=True)
            p = jnp.exp2(s - m)
            l = jnp.sum(p, axis=-1, keepdims=True)
            o = jnp.dot(p.astype(bf16), v_buf[slot][b], preferred_element_type=f32)
            r = pl.reciprocal(l, approx=True)
            r = r * (2.0 - l * r)
            o_scr[par][b * SQ:(b + 1) * SQ, :] = (o * r).astype(bf16)

        def oproj(b0, b1):
            rows = slice(b0 * SQ, b1 * SQ)
            prev = acc[br, rows, :]
            if not static and any((t * U + u) % H == 0 for t in range(NMAIN // U)):
                prev = jnp.where((j & (H - 1)) == 0, 0.0, prev)
            res = prev + jnp.dot(o_scr[par][rows, :], wo_buf[slot][...], preferred_element_type=f32)
            if last:
                ostage[1, rows, :] = res.astype(bf16)
                for b in range(b0, b1):
                    out_copy(1, b).start()
            else:
                acc[br, rows, :] = res

        if not static or j + A < NSTEP:
            qproj()
        s = scores(0)
        for b in range(B):
            s_next = scores(b + 1) if b + 1 < B else None
            pv(b, s)
            if last:
                if b >= 1:
                    oproj(b - 1, b)
            elif b == B - 2:
                oproj(0, B - 2)
            s = s_next
        if last:
            oproj(B - 1, B)
        else:
            oproj(B - 2, B)

    def body(t, carry):
        @pl.when(t == 2)
        def _():
            xb_copy.start()

        @pl.when(t == (H - A) // U)
        def _():
            xb_copy.wait()

        @pl.when(t == -(-H // U))
        def _():
            for b in range(B):
                rows = slice(b * SQ, (b + 1) * SQ)
                ostage[0, rows, :] = acc[0, rows, :].astype(bf16)
                out_copy(0, b).start()

        for u in range(U):
            step(t * U + u, u)
        return carry

    lax.fori_loop(0, NMAIN // U, body, 0)
    for j in range(NMAIN, NSTEP):
        step(j, j % U, last=(j == NSTEP - 1))
    for br in range(2):
        for b in range(B):
            out_copy(br, b).wait()


@jax.jit
def pallas_concat_heads__mha_block_cached__mha_block_cached__near_ridge_kernel(
    A_x: jax.Array,
    A_k_cache: jax.Array,
    A_v_cache: jax.Array,
    A_wq: jax.Array,
    A_wo: jax.Array,
    B_x: jax.Array,
    B_k_cache: jax.Array,
    B_v_cache: jax.Array,
    B_wq: jax.Array,
    B_wo: jax.Array,
):
    assert A_x.shape == (B, SQ, D) and A_k_cache.shape == (B, H, SK, DH)
    hbm = pl.BlockSpec(memory_space=pl.ANY)
    out = pl.pallas_call(
        _kernel,
        in_specs=[hbm] * 10,
        out_specs=hbm,
        out_shape=jax.ShapeDtypeStruct((M, 2 * D), A_x.dtype),
        scratch_shapes=[
            pltpu.VMEM((2, M, D), bf16),
            pltpu.VMEM((2, M, D), f32),
            pltpu.VMEM((2, M, D), bf16),
            pltpu.VMEM((A, D, DH), bf16),
            pltpu.VMEM((U, M, DH), bf16),
            *[pltpu.VMEM((B, SK, DH), bf16)] * NBUF,
            *[pltpu.VMEM((B, SK, DH), bf16)] * NBUF,
            *[pltpu.VMEM((D, DH), bf16)] * NBUF,
            *[pltpu.VMEM((DH, D), bf16)] * NBUF,
            *[pltpu.VMEM((M, DH), bf16)] * 2,
            pltpu.SemaphoreType.DMA((XCH + 1,)),
            pltpu.SemaphoreType.DMA((NBUF,)),
            pltpu.SemaphoreType.DMA((NBUF,)),
            pltpu.SemaphoreType.DMA((NBUF,)),
            pltpu.SemaphoreType.DMA((NBUF,)),
            pltpu.SemaphoreType.DMA((A,)),
            pltpu.SemaphoreType.DMA((2 * B,)),
        ],
        compiler_params=pltpu.CompilerParams(
            vmem_limit_bytes=64 * 1024 * 1024,
            disable_bounds_checks=True,
            flags={"XLA_TPU_RESCHEDULE_DMA_DONES": True},
        ),
        name="mha_cached_ab",
    )(A_x.reshape(M, D), A_k_cache, A_v_cache, A_wq, A_wo,
      B_x.reshape(M, D), B_k_cache, B_v_cache, B_wq, B_wo)
    return out.reshape(B, SQ, 2 * D)
```

```python
import jax
import jax.numpy as jnp
from jax import lax
import jax.experimental.pallas as pl
import jax.experimental.pallas.tpu as pltpu

B, SQ, D, H, SK, DH = 8, 160, 512, 32, 512, 128
M = B * SQ
NSTEP = 2 * H
LOG2E = 1.4426950408889634
QSCALE = (DH ** -0.5) * LOG2E

U = 6
NBUF = 6
LA = 3
A = 4
T = 4
XCH = 4
NMAIN = NSTEP - T
XR = M // XCH
XB_START = 2
XB_WAIT = (H - A) // U
assert U % NBUF == 0 and NMAIN % U == 0 and A <= T and A < U and LA < NBUF
assert T >= 4 and XB_START < XB_WAIT

K_, V_, WO_, WQ_ = range(4)
ISSUE_ORDER = (WQ_, K_, V_, WO_)

f32 = jnp.float32
bf16 = jnp.bfloat16


def _kernel(ax, ak, av, awq, awo, bx, bk, bv, bwq, bwo, out_ref, *scratch):
    scratch = list(scratch)
    take = lambda n: [scratch.pop(0) for _ in range(n)]
    x_buf, acc, wq0_buf, q_scr = take(4)
    ostage = take(2)
    k_buf, v_buf, wq_buf, wo_buf = take(NBUF), take(NBUF), take(NBUF), take(NBUF)
    o_scr = take(2)
    p_scr = take(2)
    x_sem, k_sem, v_sem, wq_sem, wo_sem, o_sem = take(6)
    srcs = ((ak, av, awq, awo), (bk, bv, bwq, bwo))

    def tile_copy(kind, br, h, slot):
        k, v, wq, wo = srcs[br]
        if kind == K_:
            return pltpu.make_async_copy(k.at[:, h], k_buf[slot], k_sem.at[slot])
        if kind == V_:
            return pltpu.make_async_copy(v.at[:, h], v_buf[slot], v_sem.at[slot])
        hs = pl.ds(pl.multiple_of(h * DH, DH), DH)
        if kind == WO_:
            return pltpu.make_async_copy(wo.at[hs, :], wo_buf[slot], wo_sem.at[slot])
        return pltpu.make_async_copy(wq.at[:, hs], wq_buf[slot], wq_sem.at[slot])

    def start_tile(kind, j, slot):
        if kind == WQ_:
            j = j + A
        if isinstance(j, int):
            if j < NSTEP:
                tile_copy(kind, j // H, j % H, slot).start()
            return
        for br in range(2):
            @pl.when((j >> 5) == br)
            def _():
                tile_copy(kind, br, j & (H - 1), slot).start()

    def wait_tile(kind, j, slot):
        if kind != WQ_ or not isinstance(j, int) or j + A < NSTEP:
            tile_copy(kind, 0, 0, slot).wait()

    def out_copy(br, b):
        sem = (k_sem, v_sem, wo_sem)[b % 3].at[NBUF + b // 3] if br == 0 else o_sem.at[b]
        rows = pl.ds(b * SQ, SQ)
        return pltpu.make_async_copy(ostage[br].at[rows, :], out_ref.at[rows, pl.ds(br * D, D)], sem)

    def xa_copy(c):
        rows = pl.ds(c * XR if isinstance(c, int) else pl.multiple_of(c * XR, XR), XR)
        return pltpu.make_async_copy(ax.at[rows, :], x_buf.at[0, rows, :], x_sem.at[c])

    xb_copy = lambda: pltpu.make_async_copy(bx, x_buf.at[1], x_sem.at[XCH])
    wq0_copy = lambda a: pltpu.make_async_copy(
        awq.at[:, pl.ds(a * DH, DH)], wq0_buf.at[a], x_sem.at[XCH + 1 + a])

    def issue(i, carry):
        @pl.when(i == 0)
        def _():
            wq0_copy(0).start()
            xa_copy(0).start()
            for a in range(1, A):
                wq0_copy(a).start()
            for c in range(1, XCH):
                xa_copy(c).start()
        for j in range(LA):
            @pl.when(i == j + 1)
            def _():
                for kind in ISSUE_ORDER:
                    start_tile(kind, j, j)
        return carry

    lax.fori_loop(0, LA + 1, issue, 0)

    def q_ahead(c, carry):
        rows = pl.ds(pl.multiple_of(c * XR, XR), XR)
        xa_copy(c).wait()
        for a in range(A):
            @pl.when(c == 0)
            def _():
                wq0_copy(a).wait()
            q = jnp.dot(x_buf[0, rows, :], wq0_buf[a], preferred_element_type=f32)
            q_scr[a, rows, :] = (q * QSCALE).astype(bf16)
        return carry

    lax.fori_loop(0, XCH, q_ahead, 0)

    def step(j, u, last=False):
        slot = u % NBUF
        par = u % 2
        static = isinstance(j, int)
        br = j // H if static else j >> 5

        def sync(kind):
            start_tile(kind, j + LA, (u + LA) % NBUF)
            wait_tile(kind, j, slot)

        def qproj():
            sync(WQ_)
            nbr = (j + A) // H if static else (j + A) >> 5
            q = jnp.dot(x_buf[nbr], wq_buf[slot][...], preferred_element_type=f32)
            q_scr[(u + A) % U] = (q * QSCALE).astype(bf16)

        def scores(b):
            return lax.dot_general(q_scr[u, b * SQ:(b + 1) * SQ, :], k_buf[slot][b],
                                   (((1,), (1,)), ((), ())), preferred_element_type=f32)

        def pv(b, s):
            m = jnp.max(s, axis=-1, keepdims=True)
            p = jnp.exp2(s - m)
            l = jnp.sum(p, axis=-1, keepdims=True)
            p_scr[b % 2][...] = p.astype(bf16)
            o = jnp.dot(p_scr[b % 2][...], v_buf[slot][b], preferred_element_type=f32)
            r = pl.reciprocal(l, approx=True)
            r = r * (2.0 - l * r)
            o_scr[par][b * SQ:(b + 1) * SQ, :] = (o * r).astype(bf16)

        def oproj(b0, b1):
            rows = slice(b0 * SQ, b1 * SQ)
            prev = acc[br, rows, :]
            if not static and any((t * U + u) % H == 0 for t in range(NMAIN // U)):
                prev = jnp.where((j & (H - 1)) == 0, 0.0, prev)
            res = prev + jnp.dot(o_scr[par][rows, :], wo_buf[slot][...], preferred_element_type=f32)
            if last:
                ostage[1][rows, :] = res.astype(bf16)
                for b in range(b0, b1):
                    out_copy(1, b).start()
            else:
                acc[br, rows, :] = res

        do_q = not static or j + A < NSTEP
        q_first = u == 0
        if do_q and q_first:
            qproj()
        sync(K_)
        s = scores(0)
        for b in range(B):
            if b == 0:
                sync(V_)
            if b == 1:
                sync(WO_)
            s_next = scores(b + 1) if b + 1 < B else None
            pv(b, s)
            if last:
                if b >= 1:
                    oproj(b - 1, b)
            elif b == B - 2:
                if do_q and not q_first:
                    qproj()
                else:
                    oproj(0, B - 2)
            s = s_next
        if last:
            oproj(B - 1, B)
        elif do_q and not q_first:
            oproj(0, B)
        else:
            oproj(B - 2, B)

    def body(t, carry):
        @pl.when(t == XB_START)
        def _():
            xb_copy().start()

        @pl.when(t == XB_WAIT)
        def _():
            xb_copy().wait()

        for u in range(U):
            step(t * U + u, u)
        return carry

    lax.fori_loop(0, NMAIN // U, body, 0)

    for j in range(NMAIN, NSTEP):
        step(j, j % U, last=(j == NSTEP - 1))
        for b in range((j - NMAIN) * 3, min(B, (j - NMAIN + 1) * 3)):
            rows = slice(b * SQ, (b + 1) * SQ)
            ostage[0][rows, :] = acc[0, rows, :].astype(bf16)
            out_copy(0, b).start()
    for br in range(2):
        for b in range(B):
            out_copy(br, b).wait()


@jax.jit
def pallas_concat_heads__mha_block_cached__mha_block_cached__near_ridge_kernel(
    A_x: jax.Array,
    A_k_cache: jax.Array,
    A_v_cache: jax.Array,
    A_wq: jax.Array,
    A_wo: jax.Array,
    B_x: jax.Array,
    B_k_cache: jax.Array,
    B_v_cache: jax.Array,
    B_wq: jax.Array,
    B_wo: jax.Array,
):
    assert A_x.shape == (B, SQ, D) and A_k_cache.shape == (B, H, SK, DH)
    hbm = pl.BlockSpec(memory_space=pl.ANY)
    out = pl.pallas_call(
        _kernel,
        in_specs=[hbm] * 10,
        out_specs=hbm,
        out_shape=jax.ShapeDtypeStruct((M, 2 * D), A_x.dtype),
        scratch_shapes=[
            pltpu.VMEM((2, M, D), bf16),
            pltpu.VMEM((2, M, D), f32),
            pltpu.VMEM((A, D, DH), bf16),
            pltpu.VMEM((U, M, DH), bf16),
            pltpu.VMEM((M, D), bf16),
            pltpu.VMEM((M, D), bf16),
            *[pltpu.VMEM((B, SK, DH), bf16)] * NBUF,
            *[pltpu.VMEM((B, SK, DH), bf16)] * NBUF,
            *[pltpu.VMEM((D, DH), bf16)] * NBUF,
            *[pltpu.VMEM((DH, D), bf16)] * NBUF,
            *[pltpu.VMEM((M, DH), bf16)] * 2,
            *[pltpu.VMEM((SQ, SK), bf16)] * 2,
            pltpu.SemaphoreType.DMA((XCH + 1 + A,)),
            pltpu.SemaphoreType.DMA((NBUF + 3,)),
            pltpu.SemaphoreType.DMA((NBUF + 3,)),
            pltpu.SemaphoreType.DMA((NBUF,)),
            pltpu.SemaphoreType.DMA((NBUF + 3,)),
            pltpu.SemaphoreType.DMA((B,)),
        ],
        compiler_params=pltpu.CompilerParams(
            vmem_limit_bytes=64 * 1024 * 1024,
            flags={"XLA_TPU_RESCHEDULE_DMA_DONES": True},
        ),
        name="mha_cached_ab",
    )(A_x.reshape(M, D), A_k_cache, A_v_cache, A_wq, A_wo,
      B_x.reshape(M, D), B_k_cache, B_v_cache, B_wq, B_wo)
    return out.reshape(B, SQ, 2 * D)
```

```python
import jax
import jax.numpy as jnp
from jax import lax
import jax.experimental.pallas as pl
import jax.experimental.pallas.tpu as pltpu

B, SQ, D, H, SK, DH = 8, 160, 512, 32, 512, 128
M = B * SQ
NSTEP = 2 * H
LOG2E = 1.4426950408889634
QSCALE = (DH ** -0.5) * LOG2E

U = 6
NBUF = 6
LA = 3
A = 4
T = 4
XCH = 4
NQF = 3
NMAIN = NSTEP - T
XR = M // XCH
XB_START = 2
XB_WAIT, XB_U = divmod(H - A, U)
XB_AT = 3
assert U % NBUF == 0 and NMAIN % U == 0 and A <= T and A < U and LA < NBUF
assert 3 * (T - 1) >= B and XB_START < XB_WAIT and XB_AT <= XB_U

K_, V_, WO_, WQ_ = range(4)
ISSUE_ORDER = (WQ_, K_, V_, WO_)

f32 = jnp.float32
bf16 = jnp.bfloat16


def _kernel(ax, ak, av, awq, awo, bx, bk, bv, bwq, bwo, out_ref, *scratch):
    scratch = list(scratch)
    take = lambda n: [scratch.pop(0) for _ in range(n)]
    x_buf, acc, wq0_buf, q_scr = take(4)
    ostage = take(2)
    k_buf, v_buf, wq_buf, wo_buf = take(NBUF), take(NBUF), take(NBUF), take(NBUF)
    o_scr = take(2)
    p_scr = take(2)
    x_sem, k_sem, v_sem, wq_sem, wo_sem, o_sem = take(6)
    srcs = ((ak, av, awq, awo), (bk, bv, bwq, bwo))

    def tile_copy(kind, br, h, slot):
        k, v, wq, wo = srcs[br]
        if kind == K_:
            return pltpu.make_async_copy(k.at[:, h], k_buf[slot], k_sem.at[slot])
        if kind == V_:
            return pltpu.make_async_copy(v.at[:, h], v_buf[slot], v_sem.at[slot])
        hs = pl.ds(pl.multiple_of(h * DH, DH), DH)
        if kind == WO_:
            return pltpu.make_async_copy(wo.at[hs, :], wo_buf[slot], wo_sem.at[slot])
        return pltpu.make_async_copy(wq.at[:, hs], wq_buf[slot], wq_sem.at[slot])

    def start_tile(kind, j, slot):
        if kind == WQ_:
            j = j + A
        if isinstance(j, int):
            if j < NSTEP:
                tile_copy(kind, j // H, j % H, slot).start()
            return
        for br in range(2):
            @pl.when((j >> 5) == br)
            def _():
                tile_copy(kind, br, j & (H - 1), slot).start()

    def wait_tile(kind, j, slot):
        if kind != WQ_ or not isinstance(j, int) or j + A < NSTEP:
            tile_copy(kind, 0, 0, slot).wait()

    def out_copy(br, b):
        sem = (k_sem, v_sem, wo_sem)[b % 3].at[NBUF] if br == 0 else o_sem.at[0]
        rows = pl.ds(b * SQ, SQ)
        return pltpu.make_async_copy(ostage[br].at[rows, :], out_ref.at[rows, pl.ds(br * D, D)], sem)

    def xa_copy(c):
        rows = pl.ds(c * XR, XR)
        return pltpu.make_async_copy(ax.at[rows, :], x_buf.at[0, rows, :], x_sem.at[c])

    xb_copy = lambda: pltpu.make_async_copy(bx, x_buf.at[1], x_sem.at[XCH])
    wq0_copy = lambda a: pltpu.make_async_copy(
        awq.at[:, pl.ds(a * DH, DH)], wq0_buf.at[a], x_sem.at[XCH + 1 + a])

    def issue(i, carry):
        @pl.when(i == 0)
        def _():
            wq0_copy(0).start()
            xa_copy(0).start()
            for a in range(1, A):
                wq0_copy(a).start()
            for c in range(1, XCH):
                xa_copy(c).start()
        for j in range(LA):
            @pl.when(i == j + 1)
            def _():
                for kind in ISSUE_ORDER:
                    start_tile(kind, j, j)
        return carry

    lax.fori_loop(0, LA + 1, issue, 0)

    for c in range(XCH):
        rows = slice(c * XR, (c + 1) * XR)
        xa_copy(c).wait()
        for a in range(A):
            if c == 0:
                wq0_copy(a).wait()
            q = jnp.dot(x_buf[0, rows, :], wq0_buf[a], preferred_element_type=f32)
            q_scr[a, rows, :] = (q * QSCALE).astype(bf16)

    def step(j, u, last=False):
        slot = u % NBUF
        par = u % 2
        static = isinstance(j, int)
        br = j // H if static else j >> 5

        def sync(kind):
            start_tile(kind, j + LA, (u + LA) % NBUF)
            wait_tile(kind, j, slot)

        def qproj():
            sync(WQ_)
            nbr = (j + A) // H if static else (j + A) >> 5
            q = jnp.dot(x_buf[nbr], wq_buf[slot][...], preferred_element_type=f32)
            q_scr[(u + A) % U] = (q * QSCALE).astype(bf16)

        def scores(b):
            return lax.dot_general(q_scr[u, b * SQ:(b + 1) * SQ, :], k_buf[slot][b],
                                   (((1,), (1,)), ((), ())), preferred_element_type=f32)

        def pv(b, s):
            m = jnp.max(s, axis=-1, keepdims=True)
            p = jnp.exp2(s - m)
            l = jnp.sum(p, axis=-1, keepdims=True)
            p_scr[b % 2][...] = p.astype(bf16)
            o = jnp.dot(p_scr[b % 2][...], v_buf[slot][b], preferred_element_type=f32)
            r = pl.reciprocal(l, approx=True)
            r = r * (2.0 - l * r)
            o_scr[par][b * SQ:(b + 1) * SQ, :] = (o * r).astype(bf16)

        def oproj(b0, b1):
            rows = slice(b0 * SQ, b1 * SQ)
            prev = acc[br, rows, :]
            if not static and any((t * U + u) % H == 0 for t in range(NMAIN // U)):
                prev = jnp.where((j & (H - 1)) == 0, 0.0, prev)
            res = prev + jnp.dot(o_scr[par][rows, :], wo_buf[slot][...], preferred_element_type=f32)
            if last:
                ostage[1][rows, :] = res.astype(bf16)
                for b in range(b0, b1):
                    out_copy(1, b).start()
            else:
                acc[br, rows, :] = res

        do_q = not static or j + A < NSTEP
        q_first = u < NQF
        if do_q and q_first:
            qproj()
        sync(K_)
        s = scores(0)
        for b in range(B):
            if b == 0:
                sync(V_)
            if b == 1:
                sync(WO_)
            s_next = scores(b + 1) if b + 1 < B else None
            pv(b, s)
            if last:
                if b >= 1:
                    oproj(b - 1, b)
            elif b == B - 2:
                if do_q and not q_first:
                    qproj()
                else:
                    oproj(0, B - 2)
            s = s_next
        if last:
            oproj(B - 1, B)
        elif do_q and not q_first:
            oproj(0, B)
        else:
            oproj(B - 2, B)

    def body(t, carry):
        for u in range(U):
            if u == XB_AT:
                @pl.when(t == XB_START)
                def _():
                    xb_copy().start()

                @pl.when(t == XB_WAIT)
                def _():
                    xb_copy().wait()

            step(t * U + u, u)
        return carry

    lax.fori_loop(0, NMAIN // U, body, 0)

    for j in range(NMAIN, NSTEP):
        step(j, j % U, last=(j == NSTEP - 1))
        for b in range((j - NMAIN) * 3, min(B, (j - NMAIN + 1) * 3)):
            rows = slice(b * SQ, (b + 1) * SQ)
            ostage[0][rows, :] = acc[0, rows, :].astype(bf16)
            out_copy(0, b).start()
    for b in range(B):
        out_copy(0, b).wait()
    pltpu.make_async_copy(ostage[1], out_ref.at[:, pl.ds(D, D)], o_sem.at[0]).wait()


@jax.jit
def pallas_concat_heads__mha_block_cached__mha_block_cached__near_ridge_kernel(
    A_x: jax.Array,
    A_k_cache: jax.Array,
    A_v_cache: jax.Array,
    A_wq: jax.Array,
    A_wo: jax.Array,
    B_x: jax.Array,
    B_k_cache: jax.Array,
    B_v_cache: jax.Array,
    B_wq: jax.Array,
    B_wo: jax.Array,
):
    assert A_x.shape == (B, SQ, D) and A_k_cache.shape == (B, H, SK, DH)
    hbm = pl.BlockSpec(memory_space=pl.ANY)
    out = pl.pallas_call(
        _kernel,
        in_specs=[hbm] * 10,
        out_specs=hbm,
        out_shape=jax.ShapeDtypeStruct((M, 2 * D), A_x.dtype),
        scratch_shapes=[
            pltpu.VMEM((2, M, D), bf16),
            pltpu.VMEM((2, M, D), f32),
            pltpu.VMEM((A, D, DH), bf16),
            pltpu.VMEM((U, M, DH), bf16),
            pltpu.VMEM((M, D), bf16),
            pltpu.VMEM((M, D), bf16),
            *[pltpu.VMEM((B, SK, DH), bf16)] * NBUF,
            *[pltpu.VMEM((B, SK, DH), bf16)] * NBUF,
            *[pltpu.VMEM((D, DH), bf16)] * NBUF,
            *[pltpu.VMEM((DH, D), bf16)] * NBUF,
            *[pltpu.VMEM((M, DH), bf16)] * 2,
            *[pltpu.VMEM((SQ, SK), bf16)] * 2,
            pltpu.SemaphoreType.DMA((XCH + 1 + A,)),
            pltpu.SemaphoreType.DMA((NBUF + 1,)),
            pltpu.SemaphoreType.DMA((NBUF + 1,)),
            pltpu.SemaphoreType.DMA((NBUF,)),
            pltpu.SemaphoreType.DMA((NBUF + 1,)),
            pltpu.SemaphoreType.DMA((1,)),
        ],
        compiler_params=pltpu.CompilerParams(
            vmem_limit_bytes=64 * 1024 * 1024,
            flags={"XLA_TPU_RESCHEDULE_DMA_DONES": True},
        ),
        name="mha_cached_ab",
    )(A_x.reshape(M, D), A_k_cache, A_v_cache, A_wq, A_wo,
      B_x.reshape(M, D), B_k_cache, B_v_cache, B_wq, B_wo)
    return out.reshape(B, SQ, 2 * D)
```

```python
import jax
import jax.numpy as jnp
from jax import lax
import jax.experimental.pallas as pl
import jax.experimental.pallas.tpu as pltpu

B, SQ, D, H, SK, DH = 8, 160, 512, 32, 512, 128
M = B * SQ
NSTEP = 2 * H
LOG2E = 1.4426950408889634
QSCALE = (DH ** -0.5) * LOG2E

U = 6
NBUF = 6
LA = 3
A = 4
T = 4
XCH = 4
SD = 2
NQF = 3
NMAIN = NSTEP - T
XR = M // XCH
XB_START = 2
XB_WAIT, XB_U = divmod(H - A, U)
XB_AT = 3
assert U % NBUF == 0 and NMAIN % U == 0 and A <= T and A < U and LA < NBUF
assert 3 * (T - 1) >= B and XB_START < XB_WAIT and XB_AT <= XB_U

K_, V_, WO_, WQ_ = range(4)
ISSUE_ORDER = (WQ_, K_, V_, WO_)

f32 = jnp.float32
bf16 = jnp.bfloat16


def _kernel(ax, ak, av, awq, awo, bx, bk, bv, bwq, bwo, out_ref, *scratch):
    scratch = list(scratch)
    take = lambda n: [scratch.pop(0) for _ in range(n)]
    x_buf, acc, wq0_buf, q_scr = take(4)
    ostage = take(2)
    k_buf, v_buf, wq_buf, wo_buf = take(NBUF), take(NBUF), take(NBUF), take(NBUF)
    o_scr = take(2)
    p_scr = take(2)
    x_sem, k_sem, v_sem, wq_sem, wo_sem, o_sem = take(6)
    srcs = ((ak, av, awq, awo), (bk, bv, bwq, bwo))

    def tile_copy(kind, br, h, slot):
        k, v, wq, wo = srcs[br]
        if kind == K_:
            return pltpu.make_async_copy(k.at[:, h], k_buf[slot], k_sem.at[slot])
        if kind == V_:
            return pltpu.make_async_copy(v.at[:, h], v_buf[slot], v_sem.at[slot])
        hs = pl.ds(pl.multiple_of(h * DH, DH), DH)
        if kind == WO_:
            return pltpu.make_async_copy(wo.at[hs, :], wo_buf[slot], wo_sem.at[slot])
        return pltpu.make_async_copy(wq.at[:, hs], wq_buf[slot], wq_sem.at[slot])

    def start_tile(kind, j, slot):
        if kind == WQ_:
            j = j + A
        if isinstance(j, int):
            if j < NSTEP:
                tile_copy(kind, j // H, j % H, slot).start()
            return
        for br in range(2):
            @pl.when((j >> 5) == br)
            def _():
                tile_copy(kind, br, j & (H - 1), slot).start()

    def wait_tile(kind, j, slot):
        if kind != WQ_ or not isinstance(j, int) or j + A < NSTEP:
            tile_copy(kind, 0, 0, slot).wait()

    def out_copy(br, b):
        sem = (k_sem, v_sem, wo_sem)[b % 3].at[NBUF] if br == 0 else o_sem.at[0]
        rows = pl.ds(b * SQ, SQ)
        return pltpu.make_async_copy(ostage[br].at[rows, :], out_ref.at[rows, pl.ds(br * D, D)], sem)

    def xa_copy(c):
        rows = pl.ds(c * XR, XR)
        return pltpu.make_async_copy(ax.at[rows, :], x_buf.at[0, rows, :], x_sem.at[c])

    xb_copy = lambda: pltpu.make_async_copy(bx, x_buf.at[1], x_sem.at[XCH])
    wq0_copy = lambda a: pltpu.make_async_copy(
        awq.at[:, pl.ds(a * DH, DH)], wq0_buf.at[a], x_sem.at[XCH + 1 + a])

    def issue(i, carry):
        @pl.when(i == 0)
        def _():
            wq0_copy(0).start()
            xa_copy(0).start()
            for a in range(1, A):
                wq0_copy(a).start()
            for c in range(1, XCH):
                xa_copy(c).start()
        for j in range(LA):
            @pl.when(i == j + 1)
            def _():
                for kind in ISSUE_ORDER:
                    start_tile(kind, j, j)
        return carry

    lax.fori_loop(0, LA + 1, issue, 0)

    for c in range(XCH):
        rows = slice(c * XR, (c + 1) * XR)
        xa_copy(c).wait()
        for a in range(A):
            if c == 0:
                wq0_copy(a).wait()
            q = jnp.dot(x_buf[0, rows, :], wq0_buf[a], preferred_element_type=f32)
            q_scr[a, rows, :] = (q * QSCALE).astype(bf16)

    def step(j, u, last=False):
        slot = u % NBUF
        par = u % 2
        static = isinstance(j, int)
        br = j // H if static else j >> 5

        def sync(kind):
            start_tile(kind, j + LA, (u + LA) % NBUF)
            wait_tile(kind, j, slot)

        def qproj():
            sync(WQ_)
            nbr = (j + A) // H if static else (j + A) >> 5
            q = jnp.dot(x_buf[nbr], wq_buf[slot][...], preferred_element_type=f32)
            q_scr[(u + A) % U] = (q * QSCALE).astype(bf16)

        def scores(b):
            return lax.dot_general(q_scr[u, b * SQ:(b + 1) * SQ, :], k_buf[slot][b],
                                   (((1,), (1,)), ((), ())), preferred_element_type=f32)

        def pv(b, s):
            m = jnp.max(s, axis=-1, keepdims=True)
            p = jnp.exp2(s - m)
            l = jnp.sum(p, axis=-1, keepdims=True)
            p_scr[b % 2][...] = p.astype(bf16)
            o = jnp.dot(p_scr[b % 2][...], v_buf[slot][b], preferred_element_type=f32)
            r = pl.reciprocal(l, approx=True)
            r = r * (2.0 - l * r)
            o_scr[par][b * SQ:(b + 1) * SQ, :] = (o * r).astype(bf16)

        def oproj(b0, b1):
            rows = slice(b0 * SQ, b1 * SQ)
            prev = acc[br, rows, :]
            if not static and any((t * U + u) % H == 0 for t in range(NMAIN // U)):
                prev = jnp.where((j & (H - 1)) == 0, 0.0, prev)
            res = prev + jnp.dot(o_scr[par][rows, :], wo_buf[slot][...], preferred_element_type=f32)
            if last:
                ostage[1][rows, :] = res.astype(bf16)
                for b in range(b0, b1):
                    out_copy(1, b).start()
            else:
                acc[br, rows, :] = res

        do_q = not static or j + A < NSTEP
        q_first = u < NQF
        if do_q and q_first:
            qproj()
        sync(K_)
        pending = [scores(b) for b in range(SD)]
        for b in range(B):
            if b == 0:
                sync(V_)
            if b == 1:
                sync(WO_)
            if b + SD < B:
                pending.append(scores(b + SD))
            pv(b, pending.pop(0))
            if last:
                if b >= 1:
                    oproj(b - 1, b)
            elif b == B - 2:
                if do_q and not q_first:
                    qproj()
                else:
                    oproj(0, B - 2)
        if last:
            oproj(B - 1, B)
        elif do_q and not q_first:
            oproj(0, B)
        else:
            oproj(B - 2, B)

    def body(t, carry):
        for u in range(U):
            if u == XB_AT:
                @pl.when(t == XB_START)
                def _():
                    xb_copy().start()

                @pl.when(t == XB_WAIT)
                def _():
                    xb_copy().wait()

            step(t * U + u, u)
        return carry

    lax.fori_loop(0, NMAIN // U, body, 0)

    for j in range(NMAIN, NSTEP):
        step(j, j % U, last=(j == NSTEP - 1))
        for b in range((j - NMAIN) * 3, min(B, (j - NMAIN + 1) * 3)):
            rows = slice(b * SQ, (b + 1) * SQ)
            ostage[0][rows, :] = acc[0, rows, :].astype(bf16)
            out_copy(0, b).start()
    for b in range(B):
        out_copy(0, b).wait()
    pltpu.make_async_copy(ostage[1], out_ref.at[:, pl.ds(D, D)], o_sem.at[0]).wait()


@jax.jit
def pallas_concat_heads__mha_block_cached__mha_block_cached__near_ridge_kernel(
    A_x: jax.Array,
    A_k_cache: jax.Array,
    A_v_cache: jax.Array,
    A_wq: jax.Array,
    A_wo: jax.Array,
    B_x: jax.Array,
    B_k_cache: jax.Array,
    B_v_cache: jax.Array,
    B_wq: jax.Array,
    B_wo: jax.Array,
):
    assert A_x.shape == (B, SQ, D) and A_k_cache.shape == (B, H, SK, DH)
    hbm = pl.BlockSpec(memory_space=pl.ANY)
    out = pl.pallas_call(
        _kernel,
        in_specs=[hbm] * 10,
        out_specs=hbm,
        out_shape=jax.ShapeDtypeStruct((M, 2 * D), A_x.dtype),
        scratch_shapes=[
            pltpu.VMEM((2, M, D), bf16),
            pltpu.VMEM((2, M, D), f32),
            pltpu.VMEM((A, D, DH), bf16),
            pltpu.VMEM((U, M, DH), bf16),
            pltpu.VMEM((M, D), bf16),
            pltpu.VMEM((M, D), bf16),
            *[pltpu.VMEM((B, SK, DH), bf16)] * NBUF,
            *[pltpu.VMEM((B, SK, DH), bf16)] * NBUF,
            *[pltpu.VMEM((D, DH), bf16)] * NBUF,
            *[pltpu.VMEM((DH, D), bf16)] * NBUF,
            *[pltpu.VMEM((M, DH), bf16)] * 2,
            *[pltpu.VMEM((SQ, SK), bf16)] * 2,
            pltpu.SemaphoreType.DMA((XCH + 1 + A,)),
            pltpu.SemaphoreType.DMA((NBUF + 1,)),
            pltpu.SemaphoreType.DMA((NBUF + 1,)),
            pltpu.SemaphoreType.DMA((NBUF,)),
            pltpu.SemaphoreType.DMA((NBUF + 1,)),
            pltpu.SemaphoreType.DMA((1,)),
        ],
        compiler_params=pltpu.CompilerParams(
            vmem_limit_bytes=64 * 1024 * 1024,
            flags={"XLA_TPU_RESCHEDULE_DMA_DONES": True},
        ),
        name="mha_cached_ab",
    )(A_x.reshape(M, D), A_k_cache, A_v_cache, A_wq, A_wo,
      B_x.reshape(M, D), B_k_cache, B_v_cache, B_wq, B_wo)
    return out.reshape(B, SQ, 2 * D)
```
